```python
import os as _os
_os.environ.setdefault("JAX_PLATFORMS", "cpu")
import jax
import jax.numpy as jnp

def _softmax(x, axis=-1):
    return jax.nn.softmax(x, axis=axis)
def _gelu(x):
    return jax.nn.gelu(x, approximate=True)
def _silu(x):
    return jax.nn.silu(x)
def _sigmoid(x):
    return jax.nn.sigmoid(x)
def _layernorm(x, axis=-1, eps=1e-5):
    m = jnp.mean(x, axis=axis, keepdims=True)
    v = jnp.var(x, axis=axis, keepdims=True)
    return (x - m) / jnp.sqrt(v + eps)
def _scatter_add(tgt, idx, src, axis=0):
    return tgt.at[idx].add(src)
def _segment_sum(src, seg, n):
    return jax.ops.segment_sum(src, seg, n)
class _Rng:
    def __init__(self, key):
        self._k = key
    def _next(self):
        self._k, sub = jax.random.split(self._k)
        return sub
    def normal(self, shape):
        return jax.random.normal(self._next(), shape, dtype=jnp.bfloat16)
    def randint(self, lo, hi, shape):
        return jax.random.randint(self._next(), shape, lo, hi, dtype=jnp.int32)
    def uniform(self, shape, lo=0.0, hi=1.0):
        return jax.random.uniform(self._next(), shape, jnp.bfloat16, lo, hi)
    def permutation(self, n):
        return jax.random.permutation(self._next(), n)


kernel_name = 'interleave_layers__mha_block__dense_activation_mish__prompt'

def setup_inputs():
    _rng = _Rng(jax.random.key(int.from_bytes(__import__("os").urandom(4), "little")))
    _w = (lambda a: (lambda t: t.astype(jnp.bfloat16) if jnp.issubdtype(t.dtype, jnp.floating) else t)(jnp.asarray(a)))
    def _A_setup():
        B, S, D, H = 1, 2048, 512, 32
        return {
            "x": _w((lambda *s: _rng.normal(s) * 0.05)(B, S, D)),
            "wqkv": _w((lambda *s: _rng.normal(s) * 0.05)(D, 3 * D)),
            "wo": _w((lambda *s: _rng.normal(s) * 0.05)(D, D)),
        }
    _A_in = _A_setup()

    def _B_setup():
        B, S, D, F = 1, 2048, 512, 1792
        return {
            "x": _w((lambda *s: _rng.normal(s) * 0.05)(B, S, D)),
            "w1": _w((lambda *s: _rng.normal(s) * 0.4)(D, F) * (D ** -0.5)),
            "b1": _w((lambda *s: _rng.normal(s) * 0.4)(F)),
            "w2": _w((lambda *s: _rng.normal(s) * 0.4)(F, D) * (F ** -0.5)),
        }
    _B_in = _B_setup()

    return {
        "A_x": _A_in["x"],
        "A_wqkv": _A_in["wqkv"],
        "A_wo": _A_in["wo"],
        "B_x": _B_in["x"],
        "B_w1": _B_in["w1"],
        "B_b1": _B_in["b1"],
        "B_w2": _B_in["w2"],
    }

def reference(A_x, A_wqkv, A_wo, B_x, B_w1, B_b1, B_w2):
    def _A_ref(x, wqkv, wo):
        B, S, D = x.shape
        H = 32
        Dh = D // H
        qkv = (lambda x, *d: x.transpose(*d))((x @ wqkv).reshape(B, S, 3, H, Dh), 2, 0, 3, 1, 4)
        q, k, v = qkv[0], qkv[1], qkv[2]
        scores = jnp.einsum("bhqd,bhkd->bhqk", q, k) * (Dh ** -0.5)
        p = _softmax(scores, axis=-1)
        o = jnp.einsum("bhqk,bhkd->bhqd", p, v)
        return (lambda x, *d: x.transpose(*d))(o, 0, 2, 1, 3).reshape(B, S, D) @ wo

    def _B_ref(x, w1, b1, w2):
        h = jnp.einsum("bsd,df->bsf", x, w1) + b1
        sp = jnp.log1p(jnp.exp(-jnp.abs(h))) + jnp.where(h > 0, h, jnp.zeros_like(h))
        act = h * jnp.tanh(sp)
        return jnp.einsum("bsf,fd->bsd", act, w2)

    x = A_x
    x = x + _A_ref(_layernorm(x, axis=-1), A_wqkv, A_wo)
    x = x + _B_ref(_layernorm(x, axis=-1), B_w1, B_b1, B_w2)
    x = x + _A_ref(_layernorm(x, axis=-1), A_wqkv, A_wo)
    x = x + _B_ref(_layernorm(x, axis=-1), B_w1, B_b1, B_w2)
    return x
```

```python
import functools
import math

import jax
import jax.numpy as jnp
from jax import lax
import jax.experimental.pallas as pl
import jax.experimental.pallas.tpu as pltpu

H = 32
DH = 16
EPS = 1e-5

TQ = 256
KC = 128
U = 4
DSK = 4

RC = 256

_LOG2E = math.log2(math.e)


def _layernorm_rows(x):
    m = jnp.mean(x, axis=-1, keepdims=True)
    xc = x - m
    v = jnp.mean(xc * xc, axis=-1, keepdims=True)
    return xc / jnp.sqrt(v + EPS)


def _kernel(x_ref, wqkv_ref, wo_ref, w1_ref, b1_ref, w2_ref, o_ref,
            xs, xn, wqT, wvT, k3, qT, vT, oT, sbuf, mbuf):
    S, D = xs.shape
    f32, bf16 = jnp.float32, jnp.bfloat16
    NQ = S // TQ
    N = H * NQ
    NK = S // KC
    L = NK + DSK
    NR = S // RC
    qscale = (DH ** -0.5) * _LOG2E

    xs[...] = x_ref[...].astype(f32)
    wqT[...] = wqkv_ref[:, 0:D].astype(f32).T.astype(bf16)
    wvT[...] = wqkv_ref[:, 2 * D:3 * D].astype(f32).T.astype(bf16)

    rows = lax.broadcasted_iota(jnp.int32, (128, TQ), 0)

    def get_qm(i):
        i = jnp.minimum(i, N - 1)
        h = i // NQ
        qi = i % NQ
        g = h // 8
        hh = h % 8
        qg = qT[pl.ds(pl.multiple_of(g * 128, 128), 128),
                pl.ds(pl.multiple_of(qi * TQ, TQ), TQ)]
        qm = jnp.where((rows >= hh * DH) & (rows < hh * DH + DH), qg,
                       jnp.zeros_like(qg))
        return qm, g

    def do_qk(qm, g, par, kc):
        sbuf[par, kc * KC:(kc + 1) * KC, :] = jnp.dot(
            k3[g, kc * KC:(kc + 1) * KC, :], qm, preferred_element_type=f32)
        if kc == NK - 1:
            mbuf[par] = jnp.max(sbuf[par], axis=0, keepdims=True)

    def attention():
        qm, g = get_qm(0)
        for kc in range(NK):
            do_qk(qm, g, 0, kc)
        qm, g = get_qm(1)
        for kc in range(DSK):
            do_qk(qm, g, 1, kc)

        def body(j, c):
            base = U * j
            qms = {}

            def qmfor(rel):
                if rel not in qms:
                    qms[rel] = get_qm(base + rel)
                return qms[rel]

            for t in range(U * NK):
                u, kc = divmod(t, NK)
                ru, rkc = divmod(t + L, NK)
                qm, g = qmfor(ru)
                do_qk(qm, g, ru % 2, rkc)
                i = base + u
                h = i // NQ
                qi = i % NQ
                ks = slice(kc * KC, (kc + 1) * KC)
                if kc == 0:
                    mc = mbuf[u % 2]
                p32 = jnp.exp2(sbuf[u % 2, ks, :] - mc)
                cl = jnp.sum(p32.reshape(KC // 8, 8, TQ), axis=0)
                p = p32.astype(bf16)
                vt = vT[pl.ds(pl.multiple_of(h * DH, DH), DH), ks]
                oo = jnp.dot(vt, p, preferred_element_type=f32)
                if kc == 0:
                    l = cl
                    o = oo
                else:
                    l = l + cl
                    o = o + oo
                if kc == NK - 1:
                    r = o / jnp.sum(l, axis=0, keepdims=True)
                    oT[pl.ds(pl.multiple_of(h * DH, DH), DH),
                       pl.ds(pl.multiple_of(qi * TQ, TQ), TQ)] = r.astype(bf16)
            return c

        lax.fori_loop(0, N // U, body, 0)

    nt = (((1,), (1,)), ((), ()))

    def layer(_, carry):
        def qkv_chunk(r, c):
            rs = pl.ds(pl.multiple_of(r * RC, RC), RC)
            xb = _layernorm_rows(xs[rs, :]).astype(bf16)
            kk = jnp.dot(xb, wqkv_ref[:, D:2 * D], preferred_element_type=f32)
            for g in range(4):
                k3[g, rs, :] = kk[:, g * 128:(g + 1) * 128].astype(bf16)
            qq = lax.dot_general(wqT[...], xb, nt, preferred_element_type=f32)
            qT[:, rs] = (qq * qscale).astype(bf16)
            vv = lax.dot_general(wvT[...], xb, nt, preferred_element_type=f32)
            vT[:, rs] = vv.astype(bf16)
            return c

        lax.fori_loop(0, NR, qkv_chunk, 0)

        attention()

        def ffn_chunk(r, c):
            rs = pl.ds(pl.multiple_of(r * RC, RC), RC)
            ob = oT[:, rs].astype(f32).T.astype(bf16)
            x1 = xs[rs, :] + jnp.dot(ob, wo_ref[...], preferred_element_type=f32)
            xb = _layernorm_rows(x1).astype(bf16)
            hh = jnp.dot(xb, w1_ref[...], preferred_element_type=f32)
            hh = hh + b1_ref[...].astype(f32)
            sp = jnp.log1p(jnp.exp(-jnp.abs(hh))) + jnp.maximum(hh, 0.0)
            act = (hh * jnp.tanh(sp)).astype(bf16)
            xs[rs, :] = x1 + jnp.dot(act, w2_ref[...], preferred_element_type=f32)
            return c

        lax.fori_loop(0, NR, ffn_chunk, 0)
        return carry

    lax.fori_loop(0, 2, layer, 0)
    o_ref[...] = xs[...].astype(o_ref.dtype)


@jax.jit
def pallas_interleave_layers__mha_block__dense_activation_mish__prompt_kernel(
    A_x: jax.Array,
    A_wqkv: jax.Array,
    A_wo: jax.Array,
    B_x: jax.Array,
    B_w1: jax.Array,
    B_b1: jax.Array,
    B_w2: jax.Array,
):
    B, S, D = A_x.shape
    F = B_w1.shape[1]
    x2 = A_x.reshape(B * S, D)
    b1 = B_b1.reshape(1, F)
    bf16, f32 = jnp.bfloat16, jnp.float32
    out = pl.pallas_call(
        _kernel,
        out_shape=jax.ShapeDtypeStruct((S, D), A_x.dtype),
        scratch_shapes=[
            pltpu.VMEM((S, D), f32),
            pltpu.VMEM((8, 128), bf16),
            pltpu.VMEM((D, D), bf16),
            pltpu.VMEM((D, D), bf16),
            pltpu.VMEM((4, S, 128), bf16),
            pltpu.VMEM((D, S), bf16),
            pltpu.VMEM((D, S), bf16),
            pltpu.VMEM((D, S), bf16),
            pltpu.VMEM((2, S, TQ), f32),
            pltpu.VMEM((2, 1, TQ), f32),
        ],
        compiler_params=pltpu.CompilerParams(
            vmem_limit_bytes=100 * 1024 * 1024),
    )(x2, A_wqkv, A_wo, B_w1, b1, B_w2)
    return out.reshape(B, S, D)
```

```python
import functools
import math

import jax
import jax.numpy as jnp
from jax import lax
import jax.experimental.pallas as pl
import jax.experimental.pallas.tpu as pltpu

H = 32
DH = 16
EPS = 1e-5

TQ = 256
KC = 128
U = 16
DSK = 4

RC = 256
ATT = 1

_LOG2E = math.log2(math.e)


def _layernorm_rows(x):
    m = jnp.mean(x, axis=-1, keepdims=True)
    xc = x - m
    v = jnp.mean(xc * xc, axis=-1, keepdims=True)
    return xc / jnp.sqrt(v + EPS)


def _kernel(x_ref, wqkv_ref, wo_hbm, w1_hbm, b1_ref, w2_hbm, o_hbm,
            xs, wqT, wvT, k3, qT, vT, oT, sbuf, mbuf,
            wo_ref, w1_ref, w2_ref, obuf, wsem, osem):
    S, D = xs.shape
    f32, bf16 = jnp.float32, jnp.bfloat16
    NQ = S // TQ
    N = H * NQ
    NK = S // KC
    L = NK + DSK
    NR = S // RC
    qscale = (DH ** -0.5) * _LOG2E

    wcopies = [
        pltpu.make_async_copy(wo_hbm, wo_ref, wsem.at[0]),
        pltpu.make_async_copy(w1_hbm, w1_ref, wsem.at[1]),
        pltpu.make_async_copy(w2_hbm, w2_ref, wsem.at[2]),
    ]
    for cp in wcopies:
        cp.start()

    def ocopy(r):
        return pltpu.make_async_copy(
            obuf.at[pl.ds(r * RC, RC), :], o_hbm.at[pl.ds(r * RC, RC), :],
            osem.at[r])

    xs[...] = x_ref[...].astype(f32)
    wqT[...] = wqkv_ref[:, 0:D].astype(f32).T.astype(bf16)
    wvT[...] = wqkv_ref[:, 2 * D:3 * D].astype(f32).T.astype(bf16)

    rows = lax.broadcasted_iota(jnp.int32, (128, TQ), 0)

    def get_qm(i):
        i = jnp.minimum(i, N - 1)
        h = i // NQ
        qi = i % NQ
        g = h // 8
        hh = h % 8
        qg = qT[pl.ds(pl.multiple_of(g * 128, 128), 128),
                pl.ds(pl.multiple_of(qi * TQ, TQ), TQ)]
        qm = jnp.where((rows >= hh * DH) & (rows < hh * DH + DH), qg,
                       jnp.zeros_like(qg))
        return qm, g

    def do_qk(qm, g, par, kc):
        sbuf[par, kc * KC:(kc + 1) * KC, :] = jnp.dot(
            k3[g, kc * KC:(kc + 1) * KC, :], qm, preferred_element_type=f32)
        if kc == NK - 1:
            mbuf[par] = jnp.max(sbuf[par], axis=0, keepdims=True)

    def attention():
        qm, g = get_qm(0)
        for kc in range(NK):
            do_qk(qm, g, 0, kc)
        qm, g = get_qm(1)
        for kc in range(DSK):
            do_qk(qm, g, 1, kc)

        def body(j, c):
            base = U * j
            qms = {}

            def qmfor(rel):
                if rel not in qms:
                    qms[rel] = get_qm(base + rel)
                return qms[rel]

            for t in range(U * NK):
                u, kc = divmod(t, NK)
                ru, rkc = divmod(t + L, NK)
                qm, g = qmfor(ru)
                do_qk(qm, g, ru % 2, rkc)
                i = base + u
                h = i // NQ
                qi = i % NQ
                ks = slice(kc * KC, (kc + 1) * KC)
                if kc == 0:
                    mc = mbuf[u % 2]
                p32 = jnp.exp2(sbuf[u % 2, ks, :] - mc)
                cl = jnp.sum(p32.reshape(KC // 8, 8, TQ), axis=0)
                p = p32.astype(bf16)
                vt = vT[pl.ds(pl.multiple_of(h * DH, DH), DH), ks]
                oo = jnp.dot(vt, p, preferred_element_type=f32)
                if kc == 0:
                    l = cl
                    o = oo
                else:
                    l = l + cl
                    o = o + oo
                if kc == NK - 1:
                    r = o / jnp.sum(l, axis=0, keepdims=True)
                    oT[pl.ds(pl.multiple_of(h * DH, DH), DH),
                       pl.ds(pl.multiple_of(qi * TQ, TQ), TQ)] = r.astype(bf16)
            return c

        lax.fori_loop(0, N // U, body, 0)

    nt = (((1,), (1,)), ((), ()))

    def layer(li, carry):
        for r in range(NR):
            rs = slice(r * RC, (r + 1) * RC)
            xb = _layernorm_rows(xs[rs, :]).astype(bf16)
            kk = jnp.dot(xb, wqkv_ref[:, D:2 * D], preferred_element_type=f32)
            for g in range(4):
                k3[g, rs, :] = kk[:, g * 128:(g + 1) * 128].astype(bf16)
            qq = lax.dot_general(wqT[...], xb, nt, preferred_element_type=f32)
            qT[:, rs] = (qq * qscale).astype(bf16)
            vv = lax.dot_general(wvT[...], xb, nt, preferred_element_type=f32)
            vT[:, rs] = vv.astype(bf16)

        if ATT:
            attention()

        @pl.when(li == 0)
        def _():
            for cp in wcopies:
                cp.wait()

        def stage_a(r):
            rs = slice(r * RC, (r + 1) * RC)
            ob = oT[:, rs].astype(f32).T.astype(bf16)
            x1 = xs[rs, :] + jnp.dot(ob, wo_ref[...], preferred_element_type=f32)
            xs[rs, :] = x1
            return _layernorm_rows(x1).astype(bf16)

        def stage_b(r, xb):
            rs = slice(r * RC, (r + 1) * RC)
            hh = jnp.dot(xb, w1_ref[...], preferred_element_type=f32)
            hh = hh + b1_ref[...].astype(f32)
            sp = jnp.log1p(jnp.exp(-jnp.abs(hh))) + jnp.maximum(hh, 0.0)
            act = (hh * jnp.tanh(sp)).astype(bf16)
            x2 = xs[rs, :] + jnp.dot(act, w2_ref[...], preferred_element_type=f32)
            xs[rs, :] = x2
            obuf[rs, :] = x2.astype(bf16)

            @pl.when(li == 1)
            def _():
                ocopy(r).start()

        xb = stage_a(0)
        for r in range(NR):
            xb_next = stage_a(r + 1) if r + 1 < NR else None
            stage_b(r, xb)
            xb = xb_next
        return carry

    lax.fori_loop(0, 2, layer, 0)
    for r in range(NR):
        ocopy(r).wait()


@jax.jit
def pallas_interleave_layers__mha_block__dense_activation_mish__prompt_kernel(
    A_x: jax.Array,
    A_wqkv: jax.Array,
    A_wo: jax.Array,
    B_x: jax.Array,
    B_w1: jax.Array,
    B_b1: jax.Array,
    B_w2: jax.Array,
):
    B, S, D = A_x.shape
    F = B_w1.shape[1]
    x2 = A_x.reshape(B * S, D)
    b1 = B_b1.reshape(1, F)
    bf16, f32 = jnp.bfloat16, jnp.float32
    out = pl.pallas_call(
        _kernel,
        out_shape=jax.ShapeDtypeStruct((S, D), A_x.dtype),
        in_specs=[
            pl.BlockSpec(memory_space=pltpu.VMEM),
            pl.BlockSpec(memory_space=pltpu.VMEM),
            pl.BlockSpec(memory_space=pl.ANY),
            pl.BlockSpec(memory_space=pl.ANY),
            pl.BlockSpec(memory_space=pltpu.VMEM),
            pl.BlockSpec(memory_space=pl.ANY),
        ],
        out_specs=pl.BlockSpec(memory_space=pl.ANY),
        scratch_shapes=[
            pltpu.VMEM((S, D), f32),
            pltpu.VMEM((D, D), bf16),
            pltpu.VMEM((D, D), bf16),
            pltpu.VMEM((4, S, 128), bf16),
            pltpu.VMEM((D, S), bf16),
            pltpu.VMEM((D, S), bf16),
            pltpu.VMEM((D, S), bf16),
            pltpu.VMEM((2, S, TQ), f32),
            pltpu.VMEM((2, 1, TQ), f32),
            pltpu.VMEM((D, D), bf16),
            pltpu.VMEM((D, F), bf16),
            pltpu.VMEM((F, D), bf16),
            pltpu.VMEM((S, D), bf16),
            pltpu.SemaphoreType.DMA((3,)),
            pltpu.SemaphoreType.DMA((S // RC,)),
        ],
        compiler_params=pltpu.CompilerParams(
            vmem_limit_bytes=100 * 1024 * 1024),
    )(x2, A_wqkv, A_wo, B_w1, b1, B_w2)
    return out.reshape(B, S, D)
```

```python
import math

import jax
import jax.numpy as jnp
from jax import lax
import jax.experimental.pallas as pl
import jax.experimental.pallas.tpu as pltpu

H = 32
DH = 16
EPS = 1e-5

TQ = 256
KC = 128
U = 32
DSK = 4
THR = 4

RC = 256

_LOG2E = math.log2(math.e)


def _layernorm_rows(x):
    m = jnp.mean(x, axis=-1, keepdims=True)
    xc = x - m
    v = jnp.mean(xc * xc, axis=-1, keepdims=True)
    return xc / jnp.sqrt(v + EPS)


def _kernel(x_ref, wqkv_ref, wo_hbm, w1_hbm, b1_ref, w2_hbm, o_hbm,
            xs, wqT, wvT, k3, qT, vT, oT, sbuf, mbuf,
            wo_ref, w1_ref, w2_ref, obuf, wsem, osem):
    S, D = xs.shape
    f32, bf16 = jnp.float32, jnp.bfloat16
    NQ = S // TQ
    N = H * NQ
    NK = S // KC
    L = NK + DSK
    NR = S // RC
    qscale = (DH ** -0.5) * _LOG2E

    wcopies = [
        pltpu.make_async_copy(wo_hbm, wo_ref, wsem.at[0]),
        pltpu.make_async_copy(w1_hbm, w1_ref, wsem.at[1]),
        pltpu.make_async_copy(w2_hbm, w2_ref, wsem.at[2]),
    ]
    for cp in wcopies:
        cp.start()

    def ocopy(r):
        return pltpu.make_async_copy(
            obuf.at[pl.ds(r * RC, RC), :], o_hbm.at[pl.ds(r * RC, RC), :],
            osem.at[r])

    xs[...] = x_ref[...].astype(f32)
    wqT[...] = wqkv_ref[:, 0:D].astype(f32).T.astype(bf16)
    wvT[...] = wqkv_ref[:, 2 * D:3 * D].astype(f32).T.astype(bf16)

    rows = lax.broadcasted_iota(jnp.int32, (128, TQ), 0)

    def get_qm(i):
        i = jnp.minimum(i, N - 1)
        h = i // NQ
        qi = i % NQ
        g = h // 8
        hh = h % 8
        qg = qT[pl.ds(pl.multiple_of(g * 128, 128), 128),
                pl.ds(pl.multiple_of(qi * TQ, TQ), TQ)]
        qm = jnp.where((rows >= hh * DH) & (rows < hh * DH + DH), qg,
                       jnp.zeros_like(qg))
        return qm, g

    hist = []

    def do_qk(qm, g, par, kc):
        s = jnp.dot(k3[g, kc * KC:(kc + 1) * KC, :], qm,
                    preferred_element_type=f32)
        sbuf[par, kc * KC:(kc + 1) * KC, :] = s
        hist.append(s[0:1, :])
        if kc == NK - 1:
            mbuf[par] = jnp.max(sbuf[par], axis=0, keepdims=True)

    def attention():
        qm, g = get_qm(0)
        for kc in range(NK):
            do_qk(qm, g, 0, kc)
        qm, g = get_qm(1)
        for kc in range(DSK):
            do_qk(qm, g, 1, kc)

        def body(j, c):
            base = U * j
            qms = {}
            hist.clear()

            def qmfor(rel):
                if rel not in qms:
                    qms[rel] = get_qm(base + rel)
                return qms[rel]

            for t in range(U * NK):
                u, kc = divmod(t, NK)
                ru, rkc = divmod(t + L, NK)
                qm, g = qmfor(ru)
                do_qk(qm, g, ru % 2, rkc)
                i = base + u
                h = i // NQ
                qi = i % NQ
                ks = slice(kc * KC, (kc + 1) * KC)
                if kc == 0:
                    mc = mbuf[u % 2]
                mct = mc
                if len(hist) > THR:
                    mct = mc + hist[-1 - THR] * 0.0
                p32 = jnp.exp2(sbuf[u % 2, ks, :] - mct)
                cl = jnp.sum(p32.reshape(KC // 8, 8, TQ), axis=0)
                p = p32.astype(bf16)
                vt = vT[pl.ds(pl.multiple_of(h * DH, DH), DH), ks]
                oo = jnp.dot(vt, p, preferred_element_type=f32)
                if kc == 0:
                    l = cl
                    o = oo
                else:
                    l = l + cl
                    o = o + oo
                if kc == NK - 1:
                    r = o / jnp.sum(l, axis=0, keepdims=True)
                    oT[pl.ds(pl.multiple_of(h * DH, DH), DH),
                       pl.ds(pl.multiple_of(qi * TQ, TQ), TQ)] = r.astype(bf16)
            return c

        lax.fori_loop(0, N // U, body, 0)

    nt = (((1,), (1,)), ((), ()))

    def layer(li, carry):
        for r in range(NR):
            rs = slice(r * RC, (r + 1) * RC)
            xb = _layernorm_rows(xs[rs, :]).astype(bf16)
            kk = jnp.dot(xb, wqkv_ref[:, D:2 * D], preferred_element_type=f32)
            for g in range(4):
                k3[g, rs, :] = kk[:, g * 128:(g + 1) * 128].astype(bf16)
            qq = lax.dot_general(wqT[...], xb, nt, preferred_element_type=f32)
            qT[:, rs] = (qq * qscale).astype(bf16)
            vv = lax.dot_general(wvT[...], xb, nt, preferred_element_type=f32)
            vT[:, rs] = vv.astype(bf16)

        attention()

        @pl.when(li == 0)
        def _():
            for cp in wcopies:
                cp.wait()

        def stage_a(r):
            rs = slice(r * RC, (r + 1) * RC)
            ob = oT[:, rs].astype(f32).T.astype(bf16)
            x1 = xs[rs, :] + jnp.dot(ob, wo_ref[...], preferred_element_type=f32)
            xs[rs, :] = x1
            return _layernorm_rows(x1).astype(bf16)

        def stage_b(r, xb):
            rs = slice(r * RC, (r + 1) * RC)
            hh = jnp.dot(xb, w1_ref[...], preferred_element_type=f32)
            hh = hh + b1_ref[...].astype(f32)
            sp = jnp.log1p(jnp.exp(-jnp.abs(hh))) + jnp.maximum(hh, 0.0)
            act = (hh * jnp.tanh(sp)).astype(bf16)
            x2 = xs[rs, :] + jnp.dot(act, w2_ref[...], preferred_element_type=f32)
            xs[rs, :] = x2
            obuf[rs, :] = x2.astype(bf16)

            @pl.when(li == 1)
            def _():
                ocopy(r).start()

        xb = stage_a(0)
        for r in range(NR):
            xb_next = stage_a(r + 1) if r + 1 < NR else None
            stage_b(r, xb)
            xb = xb_next
        return carry

    lax.fori_loop(0, 2, layer, 0)
    for r in range(NR):
        ocopy(r).wait()


@jax.jit
def pallas_interleave_layers__mha_block__dense_activation_mish__prompt_kernel(
    A_x: jax.Array,
    A_wqkv: jax.Array,
    A_wo: jax.Array,
    B_x: jax.Array,
    B_w1: jax.Array,
    B_b1: jax.Array,
    B_w2: jax.Array,
):
    B, S, D = A_x.shape
    F = B_w1.shape[1]
    x2 = A_x.reshape(B * S, D)
    b1 = B_b1.reshape(1, F)
    bf16, f32 = jnp.bfloat16, jnp.float32
    out = pl.pallas_call(
        _kernel,
        out_shape=jax.ShapeDtypeStruct((S, D), A_x.dtype),
        in_specs=[
            pl.BlockSpec(memory_space=pltpu.VMEM),
            pl.BlockSpec(memory_space=pltpu.VMEM),
            pl.BlockSpec(memory_space=pl.ANY),
            pl.BlockSpec(memory_space=pl.ANY),
            pl.BlockSpec(memory_space=pltpu.VMEM),
            pl.BlockSpec(memory_space=pl.ANY),
        ],
        out_specs=pl.BlockSpec(memory_space=pl.ANY),
        scratch_shapes=[
            pltpu.VMEM((S, D), f32),
            pltpu.VMEM((D, D), bf16),
            pltpu.VMEM((D, D), bf16),
            pltpu.VMEM((4, S, 128), bf16),
            pltpu.VMEM((D, S), bf16),
            pltpu.VMEM((D, S), bf16),
            pltpu.VMEM((D, S), bf16),
            pltpu.VMEM((2, S, TQ), f32),
            pltpu.VMEM((2, 1, TQ), f32),
            pltpu.VMEM((D, D), bf16),
            pltpu.VMEM((D, F), bf16),
            pltpu.VMEM((F, D), bf16),
            pltpu.VMEM((S, D), bf16),
            pltpu.SemaphoreType.DMA((3,)),
            pltpu.SemaphoreType.DMA((S // RC,)),
        ],
        compiler_params=pltpu.CompilerParams(
            vmem_limit_bytes=100 * 1024 * 1024),
    )(x2, A_wqkv, A_wo, B_w1, b1, B_w2)
    return out.reshape(B, S, D)
```
